```python
import os as _os
_os.environ.setdefault("JAX_PLATFORMS", "cpu")
import jax
import jax.numpy as jnp

def _softmax(x, axis=-1):
    return jax.nn.softmax(x, axis=axis)
def _gelu(x):
    return jax.nn.gelu(x, approximate=True)
def _silu(x):
    return jax.nn.silu(x)
def _sigmoid(x):
    return jax.nn.sigmoid(x)
def _layernorm(x, axis=-1, eps=1e-5):
    m = jnp.mean(x, axis=axis, keepdims=True)
    v = jnp.var(x, axis=axis, keepdims=True)
    return (x - m) / jnp.sqrt(v + eps)
def _scatter_add(tgt, idx, src, axis=0):
    return tgt.at[idx].add(src)
def _segment_sum(src, seg, n):
    return jax.ops.segment_sum(src, seg, n)
class _Rng:
    def __init__(self, key):
        self._k = key
    def _next(self):
        self._k, sub = jax.random.split(self._k)
        return sub
    def normal(self, shape):
        return jax.random.normal(self._next(), shape, dtype=jnp.bfloat16)
    def randint(self, lo, hi, shape):
        return jax.random.randint(self._next(), shape, lo, hi, dtype=jnp.int32)
    def uniform(self, shape, lo=0.0, hi=1.0):
        return jax.random.uniform(self._next(), shape, jnp.bfloat16, lo, hi)
    def permutation(self, n):
        return jax.random.permutation(self._next(), n)


kernel_name = 'interleave_layers__gqa_block_cached__dense_activation_mish__decode'

def setup_inputs():
    _rng = _Rng(jax.random.key(int.from_bytes(__import__("os").urandom(4), "little")))
    _w = (lambda a: (lambda t: t.astype(jnp.bfloat16) if jnp.issubdtype(t.dtype, jnp.floating) else t)(jnp.asarray(a)))
    def _A_setup():
        B, Sq, D = 1, 1, 512
        Hq, Hkv, Sk, Dh = 32, 8, 65536, 128
        assert Hq % Hkv == 0, (Hq, Hkv)
        return {
            "x": _w((lambda *s: _rng.normal(s) * 0.05)(B, Sq, D)),
            "k_cache": _w((lambda *s: _rng.normal(s) * 1.6)(B, Hkv, Sk, Dh)),
            "v_cache": _w((lambda *s: _rng.normal(s) * 1.6)(B, Hkv, Sk, Dh)),
            "wq": _w((lambda *s: _rng.normal(s) * 1.6)(D, Hq * Dh) * (D ** -0.5)),
            "wo": _w((lambda *s: _rng.normal(s) * 1.6)(Hq * Dh, D) * ((Hq * Dh) ** -0.5)),
        }
    _A_in = _A_setup()

    def _B_setup():
        B, S, D, F = 1, 1, 512, 1792
        return {
            "x": _w((lambda *s: _rng.normal(s) * 0.05)(B, S, D)),
            "w1": _w((lambda *s: _rng.normal(s) * 0.8)(D, F) * (D ** -0.5)),
            "b1": _w((lambda *s: _rng.normal(s) * 0.8)(F)),
            "w2": _w((lambda *s: _rng.normal(s) * 0.8)(F, D) * (F ** -0.5)),
        }
    _B_in = _B_setup()

    return {
        "A_x": _A_in["x"],
        "A_k_cache": _A_in["k_cache"],
        "A_v_cache": _A_in["v_cache"],
        "A_wq": _A_in["wq"],
        "A_wo": _A_in["wo"],
        "B_x": _B_in["x"],
        "B_w1": _B_in["w1"],
        "B_b1": _B_in["b1"],
        "B_w2": _B_in["w2"],
    }

def reference(A_x, A_k_cache, A_v_cache, A_wq, A_wo, B_x, B_w1, B_b1, B_w2):
    def _A_ref(x, k_cache, v_cache, wq, wo):
        B, Sq, D = x.shape
        Hq, Dh = 32, 128
        Hkv = k_cache.shape[1]
        rep = Hq // Hkv
        q = (lambda x, *d: x.transpose(*d))((x @ wq).reshape(B, Sq, Hq, Dh), 0, 2, 1, 3)
        k = jnp.repeat(k_cache, rep, axis=1)
        v = jnp.repeat(v_cache, rep, axis=1)
        scores = jnp.einsum("bhqd,bhkd->bhqk", q, k) * (Dh ** -0.5)
        p = _softmax(scores, axis=-1)
        o = jnp.einsum("bhqk,bhkd->bhqd", p, v)
        return (lambda x, *d: x.transpose(*d))(o, 0, 2, 1, 3).reshape(B, Sq, Hq * Dh) @ wo

    def _B_ref(x, w1, b1, w2):
        h = jnp.einsum("bsd,df->bsf", x, w1) + b1
        sp = jnp.log1p(jnp.exp(-jnp.abs(h))) + jnp.where(h > 0, h, jnp.zeros_like(h))
        act = h * jnp.tanh(sp)
        return jnp.einsum("bsf,fd->bsd", act, w2)

    x = A_x
    x = x + _A_ref(_layernorm(x, axis=-1), A_k_cache, A_v_cache, A_wq, A_wo)
    x = x + _B_ref(_layernorm(x, axis=-1), B_w1, B_b1, B_w2)
    x = x + _A_ref(_layernorm(x, axis=-1), A_k_cache, A_v_cache, A_wq, A_wo)
    x = x + _B_ref(_layernorm(x, axis=-1), B_w1, B_b1, B_w2)
    return x
```

```python
import os
import jax
import jax.numpy as jnp
from jax import lax
import jax.experimental.pallas as pl
import jax.experimental.pallas.tpu as pltpu

D_MODEL = 512
HQ = 32
HKV = 8
SK = 65536
DH = 128
FF = 1792
REP = HQ // HKV
GW = REP * DH

T = int(os.environ.get("KT", 2048))
NB = SK // T
N = HKV * NB
D = int(os.environ.get("KD", 4))
CC = int(os.environ.get("KCC", 14))
UU = NB - CC
RC = CC * HKV
M = UU * HKV
L = D - 1
SCALE = DH ** -0.5
assert CC + D <= UU


def _ln(x):
    m = jnp.mean(x, axis=-1, keepdims=True)
    xc = x - m
    v = jnp.mean(xc * xc, axis=-1, keepdims=True)
    return xc / jnp.sqrt(v + 1e-5)


def _kernel(x_hbm, k_hbm, v_hbm, wq_hbm, wo_hbm, w1_hbm, b1_hbm, w2_hbm, o_ref,
            kbuf, vbuf, x_v, wq_v, wo_v, w1_v, b1_v, w2_v, ksem, vsem, wsem):
    f32 = jnp.float32
    bf16 = jnp.bfloat16
    row = lax.broadcasted_iota(jnp.int32, (8, DH), 0)

    wcp = [pltpu.make_async_copy(src, dst, wsem.at[i]) for i, (src, dst) in enumerate(
        [(x_hbm, x_v), (wq_hbm, wq_v), (wo_hbm, wo_v), (w1_hbm, w1_v), (b1_hbm, b1_v), (w2_hbm, w2_v)])]

    def copies(b, slot, si):
        return (
            pltpu.make_async_copy(k_hbm.at[pl.ds(b * T, T)], kbuf.at[slot], ksem.at[si]),
            pltpu.make_async_copy(v_hbm.at[pl.ds(b * T, T)], vbuf.at[slot], vsem.at[si]),
        )

    def slot1(b):
        g = b // NB
        c = b % NB
        return jnp.where(c < CC, g * CC + c, RC + (g * UU + c - CC) % D)

    def copies1(b):
        return copies(b, slot1(b), b % D)

    def copies2(u):
        b = (u // UU) * NB + CC + u % UU
        return copies(b, RC + u % D, u % D)

    def start(cs):
        for c in cs:
            c.start()

    def wait(cs):
        for c in cs:
            c.wait()

    def q_head(xn, g):
        r = jnp.dot(xn, wq_v[:, g * GW:(g + 1) * GW], preferred_element_type=f32)
        qg = jnp.zeros((8, DH), f32)
        for j in range(REP):
            qg = jnp.where(row == j, r[:, j * DH:(j + 1) * DH], qg)
        return qg.astype(bf16)

    def wo_head(state, g):
        _, l, acc = state
        og = acc / l
        out = jnp.zeros((8, D_MODEL), f32)
        for j in range(REP):
            h = g * REP + j
            out = out + jnp.dot(jnp.where(row == j, og, 0.0).astype(bf16), wo_v[h * DH:(h + 1) * DH, :], preferred_element_type=f32)
        return out

    def init_state():
        return (jnp.full((8, DH), -jnp.inf, f32), jnp.zeros((8, DH), f32), jnp.zeros((8, DH), f32))

    def process(q, slot, state):
        m_old, l_old, acc = state
        s = lax.dot_general(q, kbuf[slot], (((1,), (1,)), ((), ())), preferred_element_type=f32) * SCALE
        m_new = jnp.maximum(m_old, jnp.max(s, axis=-1, keepdims=True))
        alpha = jnp.exp(m_old - m_new)
        p = jnp.exp(s - m_new[:, :1])
        l_new = alpha * l_old + jnp.sum(p, axis=-1, keepdims=True)
        pv = jnp.dot(p.astype(bf16), vbuf[slot], preferred_element_type=f32)
        return m_new, l_new, alpha * acc + pv

    def merge(sa, sb):
        m = jnp.maximum(sa[0], sb[0])
        ea = jnp.exp(sa[0] - m)
        eb = jnp.exp(sb[0] - m)
        return m, ea * sa[1] + eb * sb[1], ea * sa[2] + eb * sb[2]

    def mlp(x, first):
        xn = _ln(x).astype(bf16)
        if first:
            wcp[3].wait()
            wcp[4].wait()
        b1 = b1_v[...].astype(f32)
        bias = jnp.concatenate(
            [jnp.broadcast_to(b1[c:c + 1, :], (8, DH)) for c in range(FF // DH)], axis=1)
        h = jnp.dot(xn, w1_v[...], preferred_element_type=f32) + bias
        sp = jnp.log1p(jnp.exp(-jnp.abs(h))) + jnp.maximum(h, 0.0)
        act = h * jnp.tanh(sp)
        if first:
            wcp[5].wait()
        return x + jnp.dot(act.astype(bf16), w2_v[...], preferred_element_type=f32)

    wcp[0].start()
    wcp[1].start()
    for b in range(L):
        start(copies1(b))
    wcp[2].start()
    wcp[0].wait()
    wcp[1].wait()
    x0 = jnp.broadcast_to(x_v[...].astype(f32), (8, D_MODEL))
    xn = _ln(x0).astype(bf16)

    out8 = jnp.zeros((8, D_MODEL), f32)
    for g in range(HKV):
        q = q_head(xn, g)

        def body1(c, state, g=g, q=q):
            b = g * NB + c

            @pl.when(b + L < N)
            def _():
                start(copies1(b + L))

            if g == HKV - 1:
                @pl.when(b + L == N)
                def _():
                    for c in wcp[3:]:
                        c.start()
            wait(copies1(b))
            return process(q, slot1(b), state)

        state = lax.fori_loop(0, NB, body1, init_state())
        if g == 0:
            wcp[2].wait()
        out8 = out8 + wo_head(state, g)

    x1 = x0 + jnp.sum(out8, axis=0, keepdims=True)
    x1 = mlp(x1, True)
    xn = _ln(x1).astype(bf16)

    out8 = jnp.zeros((8, D_MODEL), f32)
    for g in reversed(range(HKV)):
        q = q_head(xn, g)

        def body_u(i, state, g=g, q=q):
            u = g * UU + (UU - 1 - i)

            @pl.when(u < M - D)
            def _():
                wait(copies2(u))
            state = process(q, RC + u % D, state)

            @pl.when(u >= D)
            def _():
                start(copies2(u - D))
            return state

        def body_uc(i, states, g=g, q=q):
            su, sc = states
            su = body_u(i, su)
            sc = process(q, g * CC + i - D, sc)
            return su, sc

        su = lax.fori_loop(0, D, body_u, init_state())
        su, sc = lax.fori_loop(D, D + CC, body_uc, (su, init_state()))
        if D + CC < UU:
            su = lax.fori_loop(D + CC, UU, body_u, su)
        state = merge(su, sc)
        out8 = out8 + wo_head(state, g)

    x2 = x1 + jnp.sum(out8, axis=0, keepdims=True)
    x2 = mlp(x2, False)
    o_ref[...] = x2[:1].astype(o_ref.dtype)


@jax.jit
def pallas_interleave_layers__gqa_block_cached__dense_activation_mish__decode_kernel(
    A_x, A_k_cache, A_v_cache, A_wq, A_wo, B_x, B_w1, B_b1, B_w2):
    x = A_x.reshape(1, D_MODEL)
    k = A_k_cache.reshape(HKV * SK, DH)
    v = A_v_cache.reshape(HKV * SK, DH)
    b1 = B_b1.reshape(FF // DH, DH)
    vm = pl.BlockSpec(memory_space=pltpu.VMEM)
    hbm = pl.BlockSpec(memory_space=pl.ANY)
    bf16 = jnp.bfloat16
    out = pl.pallas_call(
        _kernel,
        out_shape=jax.ShapeDtypeStruct((1, D_MODEL), bf16),
        in_specs=[hbm] * 8,
        out_specs=vm,
        scratch_shapes=[
            pltpu.VMEM((RC + D, T, DH), bf16),
            pltpu.VMEM((RC + D, T, DH), bf16),
            pltpu.VMEM((1, D_MODEL), bf16),
            pltpu.VMEM((D_MODEL, HQ * DH), bf16),
            pltpu.VMEM((HQ * DH, D_MODEL), bf16),
            pltpu.VMEM((D_MODEL, FF), bf16),
            pltpu.VMEM((FF // DH, DH), bf16),
            pltpu.VMEM((FF, D_MODEL), bf16),
            pltpu.SemaphoreType.DMA((D,)),
            pltpu.SemaphoreType.DMA((D,)),
            pltpu.SemaphoreType.DMA((6,)),
        ],
        compiler_params=pltpu.CompilerParams(vmem_limit_bytes=128 * 1024 * 1024),
    )(x, k, v, A_wq, A_wo, B_w1, b1, B_w2)
    return out.reshape(1, 1, D_MODEL)
```

```python
import jax
import jax.numpy as jnp
from jax import lax
import jax.experimental.pallas as pl
import jax.experimental.pallas.tpu as pltpu

D_MODEL = 512
HQ = 32
HKV = 8
SK = 65536
DH = 128
FF = 1792
REP = HQ // HKV
GW = REP * DH

T = 2048
NB = SK // T
N = HKV * NB
D = 4
CC = 14
UU = NB - CC
RC = CC * HKV
M = UU * HKV
L = D - 1
SCALE = DH ** -0.5
W2C = ((0, 768), (768, 1280), (1280, 1664), (1664, 1792))
assert CC + D <= UU


def _ln(x):
    m = jnp.mean(x, axis=-1, keepdims=True)
    xc = x - m
    v = jnp.mean(xc * xc, axis=-1, keepdims=True)
    return xc / jnp.sqrt(v + 1e-5)


def _kernel(x_hbm, k_hbm, v_hbm, wq_hbm, wo_hbm, w1_hbm, b1_hbm, w2_hbm, o_ref,
            kbuf, vbuf, x_v, wq_v, wo_v, w1_v, b1_v, w2_v, ksem, vsem, wsem):
    f32 = jnp.float32
    bf16 = jnp.bfloat16
    row = lax.broadcasted_iota(jnp.int32, (8, DH), 0)

    wcp = [pltpu.make_async_copy(src, dst, wsem.at[i]) for i, (src, dst) in enumerate(
        [(x_hbm, x_v), (wq_hbm, wq_v), (wo_hbm, wo_v), (w1_hbm, w1_v), (b1_hbm, b1_v)]
        + [(w2_hbm.at[pl.ds(lo, hi - lo)], w2_v.at[pl.ds(lo, hi - lo)]) for lo, hi in W2C])]

    def copies(b, slot, si):
        return (
            pltpu.make_async_copy(k_hbm.at[pl.ds(b * T, T)], kbuf.at[slot], ksem.at[si]),
            pltpu.make_async_copy(v_hbm.at[pl.ds(b * T, T)], vbuf.at[slot], vsem.at[si]),
        )

    def slot1(b):
        g = b // NB
        c = b % NB
        return jnp.where(c < CC, g * CC + c, RC + (g * UU + c - CC) % D)

    def copies1(b):
        return copies(b, slot1(b), b % D)

    def copies2(u):
        b = (u // UU) * NB + CC + u % UU
        return copies(b, RC + u % D, u % D)

    def q_head(xn, g):
        r = jnp.dot(xn, wq_v[:, g * GW:(g + 1) * GW], preferred_element_type=f32)
        qg = jnp.zeros((8, DH), f32)
        for j in range(REP):
            qg = jnp.where(row == j, r[:, j * DH:(j + 1) * DH], qg)
        return qg.astype(bf16)

    def wo_head(state, g):
        _, l, acc = state
        og = acc / l
        out = jnp.zeros((8, D_MODEL), f32)
        for j in range(REP):
            h = g * REP + j
            out = out + jnp.dot(jnp.where(row == j, og, 0.0).astype(bf16),
                                wo_v[h * DH:(h + 1) * DH, :], preferred_element_type=f32)
        return out

    def init_state():
        return (jnp.full((8, DH), -jnp.inf, f32), jnp.zeros((8, DH), f32),
                jnp.zeros((8, DH), f32))

    def process(q, slot, state, mid=None):
        m_old, l_old, acc = state
        s = lax.dot_general(q, kbuf[slot], (((1,), (1,)), ((), ())),
                            preferred_element_type=f32) * SCALE
        m_new = jnp.maximum(m_old, jnp.max(s, axis=-1, keepdims=True))
        alpha = jnp.exp(m_old - m_new)
        p = jnp.exp(s - m_new[:, :1])
        l_new = alpha * l_old + jnp.sum(p, axis=-1, keepdims=True)
        if mid is not None:
            mid()
        pv = jnp.dot(p.astype(bf16), vbuf[slot], preferred_element_type=f32)
        return m_new, l_new, alpha * acc + pv

    def merge(sa, sb):
        m = jnp.maximum(sa[0], sb[0])
        ea = jnp.exp(sa[0] - m)
        eb = jnp.exp(sb[0] - m)
        return m, ea * sa[1] + eb * sb[1], ea * sa[2] + eb * sb[2]

    def mlp(x, first):
        xn = _ln(x).astype(bf16)
        if first:
            wcp[3].wait()
            wcp[4].wait()
        b1 = b1_v[...].astype(f32)
        bias = jnp.concatenate(
            [jnp.broadcast_to(b1[c:c + 1, :], (8, DH)) for c in range(FF // DH)], axis=1)
        h = jnp.dot(xn, w1_v[...], preferred_element_type=f32) + bias
        sp = jnp.log1p(jnp.exp(-jnp.abs(h))) + jnp.maximum(h, 0.0)
        act = (h * jnp.tanh(sp)).astype(bf16)
        for i, (lo, hi) in enumerate(W2C):
            if first:
                wcp[5 + i].wait()
            x = x + jnp.dot(act[:, lo:hi], w2_v[lo:hi, :], preferred_element_type=f32)
        return x

    wcp[0].start()
    wcp[1].start()
    for b in range(L):
        for c in copies1(b):
            c.start()
    wcp[2].start()
    wcp[0].wait()
    wcp[1].wait()
    x0 = jnp.broadcast_to(x_v[...].astype(f32), (8, D_MODEL))
    xn = _ln(x0).astype(bf16)

    out8 = jnp.zeros((8, D_MODEL), f32)
    for g in range(HKV):
        q = q_head(xn, g)

        def body1(c, state, g=g, q=q):
            b = g * NB + c

            @pl.when(b + L < N)
            def _():
                for cp in copies1(b + L):
                    cp.start()

            if g == HKV - 1:
                @pl.when(b + L == N)
                def _():
                    for cp in wcp[3:]:
                        cp.start()
            ck, cv = copies1(b)
            ck.wait()
            return process(q, slot1(b), state, cv.wait)

        state = lax.fori_loop(0, NB, body1, init_state())
        if g == 0:
            wcp[2].wait()
        out8 = out8 + wo_head(state, g)

    x1 = x0 + jnp.sum(out8, axis=0, keepdims=True)
    x1 = mlp(x1, True)
    xn = _ln(x1).astype(bf16)

    out8 = jnp.zeros((8, D_MODEL), f32)
    for g in reversed(range(HKV)):
        q = q_head(xn, g)

        def body_u(i, state, g=g, q=q):
            u = g * UU + (UU - 1 - i)

            @pl.when(u < M - D)
            def _():
                copies2(u)[0].wait()

            def mid():
                @pl.when(u >= D)
                def _():
                    copies2(u - D)[0].start()

                @pl.when(u < M - D)
                def _():
                    copies2(u)[1].wait()
            state = process(q, RC + u % D, state, mid)

            @pl.when(u >= D)
            def _():
                copies2(u - D)[1].start()
            return state

        sh = D if g == HKV - 1 else 0

        def body_uc(i, states, g=g, q=q, sh=sh):
            su, sc = states
            su = body_u(i, su)
            sc = process(q, g * CC + i - sh, sc)
            return su, sc

        su = init_state()
        if sh:
            su = lax.fori_loop(0, sh, body_u, su)
        su, sc = lax.fori_loop(sh, sh + CC, body_uc, (su, init_state()))
        if sh + CC < UU:
            su = lax.fori_loop(sh + CC, UU, body_u, su)
        out8 = out8 + wo_head(merge(su, sc), g)

    x2 = x1 + jnp.sum(out8, axis=0, keepdims=True)
    x2 = mlp(x2, False)
    o_ref[...] = x2[:1].astype(o_ref.dtype)


@jax.jit
def pallas_interleave_layers__gqa_block_cached__dense_activation_mish__decode_kernel(
    A_x: jax.Array,
    A_k_cache: jax.Array,
    A_v_cache: jax.Array,
    A_wq: jax.Array,
    A_wo: jax.Array,
    B_x: jax.Array,
    B_w1: jax.Array,
    B_b1: jax.Array,
    B_w2: jax.Array,
):
    del B_x
    x = A_x.reshape(1, D_MODEL)
    k = A_k_cache.reshape(HKV * SK, DH)
    v = A_v_cache.reshape(HKV * SK, DH)
    b1 = B_b1.reshape(FF // DH, DH)
    vm = pl.BlockSpec(memory_space=pltpu.VMEM)
    hbm = pl.BlockSpec(memory_space=pl.ANY)
    bf16 = jnp.bfloat16
    out = pl.pallas_call(
        _kernel,
        out_shape=jax.ShapeDtypeStruct((1, D_MODEL), bf16),
        in_specs=[hbm] * 8,
        out_specs=vm,
        scratch_shapes=[
            pltpu.VMEM((RC + D, T, DH), bf16),
            pltpu.VMEM((RC + D, T, DH), bf16),
            pltpu.VMEM((1, D_MODEL), bf16),
            pltpu.VMEM((D_MODEL, HQ * DH), bf16),
            pltpu.VMEM((HQ * DH, D_MODEL), bf16),
            pltpu.VMEM((D_MODEL, FF), bf16),
            pltpu.VMEM((FF // DH, DH), bf16),
            pltpu.VMEM((FF, D_MODEL), bf16),
            pltpu.SemaphoreType.DMA((D,)),
            pltpu.SemaphoreType.DMA((D,)),
            pltpu.SemaphoreType.DMA((5 + len(W2C),)),
        ],
        compiler_params=pltpu.CompilerParams(vmem_limit_bytes=128 * 1024 * 1024),
    )(x, k, v, A_wq, A_wo, B_w1, b1, B_w2)
    return out.reshape(1, 1, D_MODEL)
```

```python
import jax
import jax.numpy as jnp
from jax import lax
import jax.experimental.pallas as pl
import jax.experimental.pallas.tpu as pltpu

D_MODEL = 512
HQ = 32
HKV = 8
SK = 65536
DH = 128
FF = 1792
REP = HQ // HKV
GW = REP * DH

T = 2048
NB = SK // T
N = HKV * NB
D = 4
CC = 14
UU = NB - CC
RC = CC * HKV
M = UU * HKV
L = D - 1
SCALE = DH ** -0.5
W2C = ((0, 768), (768, 1280), (1280, 1664), (1664, 1792))
assert CC + D <= UU


def _ln(x):
    m = jnp.mean(x, axis=-1, keepdims=True)
    xc = x - m
    v = jnp.mean(xc * xc, axis=-1, keepdims=True)
    return xc / jnp.sqrt(v + 1e-5)


def _kernel(x_hbm, k_hbm, v_hbm, wq_hbm, wo_hbm, w1_hbm, b1_hbm, w2_hbm, o_ref,
            kbuf, vbuf, x_v, wq_v, wo_v, w1_v, b1_v, w2_v, ksem, vsem, wsem):
    f32 = jnp.float32
    bf16 = jnp.bfloat16
    row = lax.broadcasted_iota(jnp.int32, (8, DH), 0)

    wcp = [pltpu.make_async_copy(src, dst, wsem.at[i]) for i, (src, dst) in enumerate(
        [(x_hbm, x_v), (wq_hbm, wq_v), (wo_hbm, wo_v), (w1_hbm, w1_v), (b1_hbm, b1_v)]
        + [(w2_hbm.at[pl.ds(lo, hi - lo)], w2_v.at[pl.ds(lo, hi - lo)]) for lo, hi in W2C])]

    def kcopy(b, slot, si):
        return pltpu.make_async_copy(k_hbm.at[pl.ds(b * T, T)], kbuf.at[slot], ksem.at[si])

    def vcopy(b, slot, si):
        return pltpu.make_async_copy(v_hbm.at[pl.ds(b * T, T)], vbuf.at[slot], vsem.at[si])

    def slot1(b):
        g = b // NB
        c = b % NB
        return jnp.where(c < CC, g * CC + c, RC + (g * UU + c - CC) % D)

    def copies1(b):
        return kcopy(b, slot1(b), b % D), vcopy(b, slot1(b), b % D)

    def copy2(fn, u):
        return fn((u // UU) * NB + CC + u % UU, RC + u % D, u % D)

    def q_head(xn, g):
        r = jnp.dot(xn, wq_v[:, g * GW:(g + 1) * GW], preferred_element_type=f32)
        qg = jnp.zeros((8, DH), f32)
        for j in range(REP):
            qg = jnp.where(row == j, r[:, j * DH:(j + 1) * DH], qg)
        return qg.astype(bf16)

    def wo_head(state, g):
        _, l, acc = state
        og = acc / l
        out = jnp.zeros((8, D_MODEL), f32)
        for j in range(REP):
            h = g * REP + j
            out = out + jnp.dot(jnp.where(row == j, og, 0.0).astype(bf16),
                                wo_v[h * DH:(h + 1) * DH, :], preferred_element_type=f32)
        return out

    def init_state():
        return (jnp.full((8, DH), -jnp.inf, f32), jnp.zeros((8, DH), f32),
                jnp.zeros((8, DH), f32))

    def process(q, slot, state, mid=None):
        m_old, l_old, acc = state
        s = lax.dot_general(q, kbuf[slot], (((1,), (1,)), ((), ())),
                            preferred_element_type=f32) * SCALE
        m_new = jnp.maximum(m_old, jnp.max(s, axis=-1, keepdims=True))
        alpha = jnp.exp(m_old - m_new)
        p = jnp.exp(s - m_new[:, :1])
        l_new = alpha * l_old + jnp.sum(p, axis=-1, keepdims=True)
        if mid is not None:
            mid()
        pv = jnp.dot(p.astype(bf16), vbuf[slot], preferred_element_type=f32)
        return m_new, l_new, alpha * acc + pv

    def merge(sa, sb):
        m = jnp.maximum(sa[0], sb[0])
        ea = jnp.exp(sa[0] - m)
        eb = jnp.exp(sb[0] - m)
        return m, ea * sa[1] + eb * sb[1], ea * sa[2] + eb * sb[2]

    def mlp(x, first):
        xn = _ln(x).astype(bf16)
        if first:
            wcp[3].wait()
            wcp[4].wait()
        b1 = b1_v[...].astype(f32)
        bias = jnp.concatenate(
            [jnp.broadcast_to(b1[c:c + 1, :], (8, DH)) for c in range(FF // DH)], axis=1)
        h = jnp.dot(xn, w1_v[...], preferred_element_type=f32) + bias
        sp = jnp.log1p(jnp.exp(-jnp.abs(h))) + jnp.maximum(h, 0.0)
        act = (h * jnp.tanh(sp)).astype(bf16)
        for i, (lo, hi) in enumerate(W2C):
            if first:
                wcp[5 + i].wait()
            x = x + jnp.dot(act[:, lo:hi], w2_v[lo:hi, :], preferred_element_type=f32)
        return x

    wcp[0].start()
    wcp[1].start()
    for b in range(L):
        for c in copies1(b):
            c.start()
    wcp[2].start()
    wcp[0].wait()
    wcp[1].wait()
    x0 = jnp.broadcast_to(x_v[...].astype(f32), (8, D_MODEL))
    xn = _ln(x0).astype(bf16)

    out8 = jnp.zeros((8, D_MODEL), f32)
    for g in range(HKV):
        q = q_head(xn, g)

        def body1(c, state, g=g, q=q):
            b = g * NB + c

            @pl.when(b + L < N)
            def _():
                for cp in copies1(b + L):
                    cp.start()

            if g == HKV - 1:
                @pl.when(b + L == N)
                def _():
                    for cp in wcp[3:]:
                        cp.start()
            ck, cv = copies1(b)
            ck.wait()
            return process(q, slot1(b), state, cv.wait)

        state = lax.fori_loop(0, NB, body1, init_state())
        if g == 0:
            wcp[2].wait()
        out8 = out8 + wo_head(state, g)

    x1 = x0 + jnp.sum(out8, axis=0, keepdims=True)
    x1 = mlp(x1, True)
    xn = _ln(x1).astype(bf16)

    out8 = jnp.zeros((8, D_MODEL), f32)
    for g in reversed(range(HKV)):
        q = q_head(xn, g)

        def body_u(i, state, g=g, q=q):
            u = g * UU + (UU - 1 - i)

            @pl.when(u < M - D)
            def _():
                copy2(kcopy, u).wait()

            def mid():
                @pl.when(u >= D)
                def _():
                    copy2(kcopy, u - D).start()

                @pl.when(u < M - D)
                def _():
                    copy2(vcopy, u).wait()
            state = process(q, RC + u % D, state, mid)

            @pl.when(u >= D)
            def _():
                copy2(vcopy, u - D).start()
            return state

        sh = D if g == HKV - 1 else 0

        def body_uc(i, states, g=g, q=q, sh=sh):
            su, sc = states
            su = body_u(i, su)
            sc = process(q, g * CC + i - sh, sc)
            return su, sc

        su = init_state()
        if sh:
            su = lax.fori_loop(0, sh, body_u, su)
        su, sc = lax.fori_loop(sh, sh + CC, body_uc, (su, init_state()))
        if sh + CC < UU:
            su = lax.fori_loop(sh + CC, UU, body_u, su)
        out8 = out8 + wo_head(merge(su, sc), g)

    x2 = x1 + jnp.sum(out8, axis=0, keepdims=True)
    x2 = mlp(x2, False)
    o_ref[...] = x2[:1].astype(o_ref.dtype)


@jax.jit
def pallas_interleave_layers__gqa_block_cached__dense_activation_mish__decode_kernel(
    A_x: jax.Array,
    A_k_cache: jax.Array,
    A_v_cache: jax.Array,
    A_wq: jax.Array,
    A_wo: jax.Array,
    B_x: jax.Array,
    B_w1: jax.Array,
    B_b1: jax.Array,
    B_w2: jax.Array,
):
    del B_x
    x = A_x.reshape(1, D_MODEL)
    k = A_k_cache.reshape(HKV * SK, DH)
    v = A_v_cache.reshape(HKV * SK, DH)
    b1 = B_b1.reshape(FF // DH, DH)
    vm = pl.BlockSpec(memory_space=pltpu.VMEM)
    hbm = pl.BlockSpec(memory_space=pl.ANY)
    bf16 = jnp.bfloat16
    out = pl.pallas_call(
        _kernel,
        out_shape=jax.ShapeDtypeStruct((1, D_MODEL), bf16),
        in_specs=[hbm] * 8,
        out_specs=vm,
        scratch_shapes=[
            pltpu.VMEM((RC + D, T, DH), bf16),
            pltpu.VMEM((RC + D, T, DH), bf16),
            pltpu.VMEM((1, D_MODEL), bf16),
            pltpu.VMEM((D_MODEL, HQ * DH), bf16),
            pltpu.VMEM((HQ * DH, D_MODEL), bf16),
            pltpu.VMEM((D_MODEL, FF), bf16),
            pltpu.VMEM((FF // DH, DH), bf16),
            pltpu.VMEM((FF, D_MODEL), bf16),
            pltpu.SemaphoreType.DMA((D,)),
            pltpu.SemaphoreType.DMA((D,)),
            pltpu.SemaphoreType.DMA((5 + len(W2C),)),
        ],
        compiler_params=pltpu.CompilerParams(vmem_limit_bytes=128 * 1024 * 1024),
    )(x, k, v, A_wq, A_wo, B_w1, b1, B_w2)
    return out.reshape(1, 1, D_MODEL)
```
